```python
import os as _os
_os.environ.setdefault("JAX_PLATFORMS", "cpu")
import jax
import jax.numpy as jnp

def _softmax(x, axis=-1):
    return jax.nn.softmax(x, axis=axis)
def _gelu(x):
    return jax.nn.gelu(x, approximate=True)
def _silu(x):
    return jax.nn.silu(x)
def _sigmoid(x):
    return jax.nn.sigmoid(x)
def _layernorm(x, axis=-1, eps=1e-5):
    m = jnp.mean(x, axis=axis, keepdims=True)
    v = jnp.var(x, axis=axis, keepdims=True)
    return (x - m) / jnp.sqrt(v + eps)
def _scatter_add(tgt, idx, src, axis=0):
    return tgt.at[idx].add(src)
def _segment_sum(src, seg, n):
    return jax.ops.segment_sum(src, seg, n)
class _Rng:
    def __init__(self, key):
        self._k = key
    def _next(self):
        self._k, sub = jax.random.split(self._k)
        return sub
    def normal(self, shape):
        return jax.random.normal(self._next(), shape, dtype=jnp.bfloat16)
    def randint(self, lo, hi, shape):
        return jax.random.randint(self._next(), shape, lo, hi, dtype=jnp.int32)
    def uniform(self, shape, lo=0.0, hi=1.0):
        return jax.random.uniform(self._next(), shape, jnp.bfloat16, lo, hi)
    def permutation(self, n):
        return jax.random.permutation(self._next(), n)


kernel_name = 'concat_heads__mha_block__linear_attn_block__prompt'

def setup_inputs():
    _rng = _Rng(jax.random.key(int.from_bytes(__import__("os").urandom(4), "little")))
    _w = (lambda a: (lambda t: t.astype(jnp.bfloat16) if jnp.issubdtype(t.dtype, jnp.floating) else t)(jnp.asarray(a)))
    def _A_setup():
        B, S, D, H = 1, 2048, 1024, 32
        return {
            "x": _w((lambda *s: _rng.normal(s) * 0.2)(B, S, D)),
            "wqkv": _w((lambda *s: _rng.normal(s) * 0.2)(D, 3 * D)),
            "wo": _w((lambda *s: _rng.normal(s) * 0.05)(D, D)),
        }
    _A_in = _A_setup()

    def _B_setup():
        B, S, D = 1, 2048, 1024
        return {
            "x": _w((lambda *s: _rng.normal(s) * 0.05)(B, S, D)),
            "wqkv": _w((lambda *s: _rng.normal(s) * 1.6)(D, 3 * D)),
            "wo": _w((lambda *s: _rng.normal(s) * 0.1)(D, D)),
        }
    _B_in = _B_setup()

    return {
        "A_x": _A_in["x"],
        "A_wqkv": _A_in["wqkv"],
        "A_wo": _A_in["wo"],
        "B_x": _B_in["x"],
        "B_wqkv": _B_in["wqkv"],
        "B_wo": _B_in["wo"],
    }

def reference(A_x, A_wqkv, A_wo, B_x, B_wqkv, B_wo):
    def _A_ref(x, wqkv, wo):
        B, S, D = x.shape
        H = 32
        Dh = D // H
        qkv = (lambda x, *d: x.transpose(*d))((x @ wqkv).reshape(B, S, 3, H, Dh), 2, 0, 3, 1, 4)
        q, k, v = qkv[0], qkv[1], qkv[2]
        scores = jnp.einsum("bhqd,bhkd->bhqk", q, k) * (Dh ** -0.5)
        p = _softmax(scores, axis=-1)
        o = jnp.einsum("bhqk,bhkd->bhqd", p, v)
        return (lambda x, *d: x.transpose(*d))(o, 0, 2, 1, 3).reshape(B, S, D) @ wo

    def _B_ref(x, wqkv, wo):
        B, S, D = x.shape
        H = 32; Dh = D // H
        qkv = (lambda x, *d: x.transpose(*d))((x @ wqkv).reshape(B, S, 3, H, Dh), 2, 0, 3, 1, 4)
        q, k, v = qkv[0], qkv[1], qkv[2]
        phi = lambda t: jnp.where(t > 0, t + 1, jnp.exp(t)) + 1e-6
        pq, pk = phi(q), phi(k)
        kv = jnp.einsum("bhsd,bhse->bhde", pk, v)
        z = jnp.einsum("bhsd->bhd", pk)
        num = jnp.einsum("bhqd,bhde->bhqe", pq, kv)
        den = jnp.einsum("bhqd,bhd->bhq", pq, z)[..., None] + 1e-6
        o = num / den
        return (lambda x, *d: x.transpose(*d))(o, 0, 2, 1, 3).reshape(B, S, D) @ wo

    a = _A_ref(A_x, A_wqkv, A_wo)
    b = _B_ref(B_x, B_wqkv, B_wo)
    return jnp.concatenate([a, b], axis=-1)
```

```python
import numpy as np
import jax
import jax.numpy as jnp
import jax.experimental.pallas as pl
import jax.experimental.pallas.tpu as pltpu

S = 2048
D = 1024
H = 32
DH = D // H
HG = 8
CK = 256
BQ = 2048
RB = 512

_NN = (((1,), (0,)), ((), ()))
_NT = (((1,), (1,)), ((), ()))
_TN = (((0,), (0,)), ((), ()))
_QSCALE = float(DH ** -0.5 * np.log2(np.e))
_SAFE = float(2.0 ** 80)
BF = jnp.bfloat16
F32 = jnp.float32


def _dot(a, b, dims):
    return jax.lax.dot_general(a, b, dims, preferred_element_type=F32)


def _phi(t):
    return jnp.where(t > 0, t + 1.0, jnp.exp(t)) + 1e-6


def _kernel(ax_h, aw_h, awo_h, bx_h, bw_h, bwo_h, out_h,
            xa, wa, woa, xb, wb, wob,
            k_s, q_s, wt0, wt1, vt_s, ot_s, m_s, z_s, in_sem, out_sem):
    nrb = S // RB

    cps = {}
    order = []

    def add(name, src, dst):
        cps[name] = pltpu.make_async_copy(src, dst, in_sem.at[len(order)])
        order.append(name)

    add("xa0", ax_h.at[0, pl.ds(0, RB), :], xa.at[pl.ds(0, RB), :])
    add("wak", aw_h.at[:, pl.ds(D, D)], wa.at[:, pl.ds(D, D)])
    add("waq", aw_h.at[:, pl.ds(0, D)], wa.at[:, pl.ds(0, D)])
    for r in range(1, nrb):
        add(f"xa{r}", ax_h.at[0, pl.ds(r * RB, RB), :], xa.at[pl.ds(r * RB, RB), :])
    add("wav", aw_h.at[:, pl.ds(2 * D, D)], wa.at[:, pl.ds(2 * D, D)])
    add("woa", awo_h, woa)
    add("xb", bx_h.at[0], xb)
    add("wb", bw_h, wb)
    add("wob", bwo_h, wob)
    for name in order:
        cps[name].start()

    cps["xa0"].wait()
    cps["wak"].wait()
    for r in range(nrb):
        rows = pl.ds(r * RB, RB)
        if r > 0:
            cps[f"xa{r}"].wait()
        x = xa[rows, :]
        kk = _dot(x, wa[:, D:2 * D], _NN).astype(BF)
        for g in range(HG):
            k_s[g, rows, :] = kk[:, g * 128:(g + 1) * 128]
        if r == 0:
            cps["waq"].wait()
        qq = (_dot(x, wa[:, 0:D], _NN) * _QSCALE).astype(BF)
        for g in range(HG):
            q_s[g, rows, :] = qq[:, g * 128:(g + 1) * 128]
    cps["wav"].wait()
    wt0[...] = wa[:, 2 * D:3 * D].T
    for r in range(nrb):
        vt_s[:, r * RB:(r + 1) * RB] = _dot(wt0[...], xa[r * RB:(r + 1) * RB, :], _NT).astype(BF)

    nck = S // CK
    nqb = S // BQ

    def q_weights(h, qb):
        blk = q_s[h // 4, pl.ds(pl.multiple_of(qb * BQ, BQ), BQ), :]
        lane = jax.lax.broadcasted_iota(jnp.int32, (BQ, 128), 1)
        return jnp.where((lane >> 5) == h % 4, blk, jnp.zeros_like(blk))

    def fast_body(it, chk):
        qb = it // H
        h = it % H
        hg = h // 4
        r0 = pl.multiple_of(h * DH, DH)
        wq = q_weights(h, qb)

        def qk(c):
            return _dot(k_s[hg, c * CK:(c + 1) * CK, :], wq, _NT)

        def pv(c, pb):
            return _dot(vt_s[pl.ds(r0, DH), c * CK:(c + 1) * CK], pb, _NN)

        s = qk(0)
        pb = acc = l = m = None
        for c in range(nck):
            sn = qk(c + 1) if c + 1 < nck else None
            if pb is not None:
                a = pv(c - 1, pb)
                acc = a if acc is None else acc + a
            s3 = s.reshape(CK // 8, 8, BQ)
            if c == 0:
                m = jnp.broadcast_to(
                    jnp.max(jnp.max(s3, axis=0), axis=0, keepdims=True), (8, BQ))
            p = jnp.exp2(s3 - m[None])
            ls = jnp.sum(p, axis=0)
            l = ls if l is None else l + ls
            pb = p.reshape(CK, BQ).astype(BF)
            s = sn
        acc = acc + pv(nck - 1, pb)
        lt = jnp.sum(l, axis=0, keepdims=True)
        o = acc * (1.0 / lt)
        ot_s[pl.ds(r0, DH), pl.ds(pl.multiple_of(qb * BQ, BQ), BQ)] = o.astype(BF)
        return chk + jnp.sum(jnp.abs(o).reshape(DH // 8, 8, BQ), axis=0) + lt

    chk = jax.lax.fori_loop(0, nqb * H, fast_body, jnp.zeros((8, BQ), F32))
    n_bad = jnp.sum(jnp.where(chk < _SAFE, 0.0, 1.0))

    @pl.when(n_bad > 0.0)
    def _exact_max_path():
        SB = 512

        def body(it, _):
            qb = it // H
            h = it % H
            hg = h // 4
            r0 = pl.multiple_of(h * DH, DH)
            cols = pl.ds(pl.multiple_of(qb * SB, SB), SB)
            blk = q_s[hg, cols, :]
            lane = jax.lax.broadcasted_iota(jnp.int32, (SB, 128), 1)
            wq = jnp.where((lane >> 5) == h % 4, blk, jnp.zeros_like(blk))

            def qk(c):
                return _dot(k_s[hg, pl.ds(pl.multiple_of(c * CK, CK), CK), :], wq, _NT)

            def mx(c, m):
                return jnp.maximum(m, jnp.max(qk(c), axis=0, keepdims=True))

            m = jax.lax.fori_loop(0, nck, mx, jnp.full((1, SB), -jnp.inf, F32))

            def ac(c, carry):
                acc, l = carry
                p = jnp.exp2(qk(c) - m)
                vt = vt_s[pl.ds(r0, DH), pl.ds(pl.multiple_of(c * CK, CK), CK)]
                return (acc + _dot(vt, p.astype(BF), _NN),
                        l + jnp.sum(p, axis=0, keepdims=True))

            acc, l = jax.lax.fori_loop(
                0, nck, ac, (jnp.zeros((DH, SB), F32), jnp.zeros((1, SB), F32)))
            ot_s[pl.ds(r0, DH), cols] = (acc / l).astype(BF)
            return 0

        jax.lax.fori_loop(0, (S // SB) * H, body, 0)

    def store_out(stage, r, y, col0, sem):
        rows = pl.ds(r * RB, RB)
        outs = []
        for g in range(HG):
            stage[g, rows, :] = y[:, g * 128:(g + 1) * 128]
        for g in range(HG):
            cp = pltpu.make_async_copy(
                stage.at[g, rows, :],
                out_h.at[0, rows, pl.ds(col0 + g * 128, 128)], out_sem.at[sem])
            cp.start()
            outs.append(cp)
        return outs

    out_cps = []
    cps["woa"].wait()
    for r in range(nrb):
        y = _dot(ot_s[:, r * RB:(r + 1) * RB], woa[...], _TN).astype(BF)
        out_cps += store_out(k_s, r, y, 0, r)

    cps["xb"].wait()
    cps["wb"].wait()
    cps["wob"].wait()
    wt0[...] = wb[:, D:2 * D].T
    wt1[...] = wb[:, 0:D].T
    pkt = vt_s
    zacc = None
    for r in range(nrb):
        pk = _phi(_dot(wt0[...], xb[r * RB:(r + 1) * RB, :], _NT))
        pkt[:, r * RB:(r + 1) * RB] = pk.astype(BF)
        for j in range(RB // 128):
            t = pk[:, j * 128:(j + 1) * 128]
            zacc = t if zacc is None else zacc + t
    z_s[...] = jnp.broadcast_to(jnp.sum(zacc, axis=1, keepdims=True), (D, 128))

    row = jax.lax.broadcasted_iota(jnp.int32, (128, 128), 0)
    col = jax.lax.broadcasted_iota(jnp.int32, (128, 128), 1)
    diag = (row >> 5) == (col >> 5)
    for r in range(D // RB):
        gm = _dot(pkt[r * RB:(r + 1) * RB, :], xb[...], _NN).astype(BF)
        for j in range(RB // 128):
            g = r * (RB // 128) + j
            kv = _dot(gm[j * 128:(j + 1) * 128, :],
                      wb[:, 2 * D + g * 128:2 * D + (g + 1) * 128], _NN)
            kv = jnp.where(diag, kv, 0.0).astype(BF)
            m_s[g * 128:(g + 1) * 128, :] = _dot(
                kv, wob[g * 128:(g + 1) * 128, :], _NN).astype(BF)

    pqt = ot_s
    for r in range(nrb):
        pq = _phi(_dot(wt1[...], xb[r * RB:(r + 1) * RB, :], _NT))
        zz = z_s[...]
        for j in range(RB // 128):
            t = pq[:, j * 128:(j + 1) * 128]
            den = jnp.sum((t * zz).reshape(H, DH, 128), axis=1, keepdims=True) + 1e-6
            tn = t.reshape(H, DH, 128) * (1.0 / den)
            pqt[:, r * RB + j * 128:r * RB + (j + 1) * 128] = tn.reshape(D, 128).astype(BF)
    for r in range(nrb):
        y = _dot(pqt[:, r * RB:(r + 1) * RB], m_s[...], _TN).astype(BF)
        out_cps += store_out(q_s, r, y, D, nrb + r)

    for cp in out_cps:
        cp.wait()


@jax.jit
def pallas_concat_heads__mha_block__linear_attn_block__prompt_kernel(
    A_x: jax.Array,
    A_wqkv: jax.Array,
    A_wo: jax.Array,
    B_x: jax.Array,
    B_wqkv: jax.Array,
    B_wo: jax.Array,
):
    hbm = pl.BlockSpec(memory_space=pl.ANY)
    return pl.pallas_call(
        _kernel,
        in_specs=[hbm] * 6,
        out_specs=hbm,
        out_shape=jax.ShapeDtypeStruct((1, S, 2 * D), BF),
        scratch_shapes=[
            pltpu.VMEM((S, D), BF), pltpu.VMEM((D, 3 * D), BF), pltpu.VMEM((D, D), BF),
            pltpu.VMEM((S, D), BF), pltpu.VMEM((D, 3 * D), BF), pltpu.VMEM((D, D), BF),
            pltpu.VMEM((HG, S, 128), BF), pltpu.VMEM((HG, S, 128), BF),
            pltpu.VMEM((D, D), BF), pltpu.VMEM((D, D), BF),
            pltpu.VMEM((D, S), BF), pltpu.VMEM((D, S), BF),
            pltpu.VMEM((D, D), BF), pltpu.VMEM((D, 128), F32),
            pltpu.SemaphoreType.DMA((16,)), pltpu.SemaphoreType.DMA((8,)),
        ],
        compiler_params=pltpu.CompilerParams(vmem_limit_bytes=110 * 2 ** 20),
    )(A_x, A_wqkv, A_wo, B_x, B_wqkv, B_wo)
```

```python
import numpy as np
import jax
import jax.numpy as jnp
import jax.experimental.pallas as pl
import jax.experimental.pallas.tpu as pltpu

S = 2048
D = 1024
H = 32
DH = D // H
HG = H // 4
S2 = S // 2
D2 = D // 2
CK = 256
HU = 2
RB = 256
NRB = S2 // RB
TR = 128

_NN = (((1,), (0,)), ((), ()))
_NT = (((1,), (1,)), ((), ()))
_QSCALE = float(DH ** -0.5 * np.log2(np.e))
_SAFE = float(2.0 ** 120)
BF = jnp.bfloat16
F32 = jnp.float32
I32 = jnp.int32

_SUMS = {"P": (0, 3, 1), "Q": (2, 3, 1), "R": (0, 1, 1), "T": (2, 0, -1), "U": (1, 3, -1)}
_SLOT = {"P": 0, "Q": 1, "R": 2, "T": 3, "U": 4, "11": 5, "22": 6}


def _dot(a, b, dims=_NN):
    return jax.lax.dot_general(a, b, dims, preferred_element_type=F32)


def _dot_t(a, bt):
    return _dot(bt, a, _NT)


def _pack(x):
    return pltpu.bitcast(x.astype(BF), I32)


def _unpack(x):
    return pltpu.bitcast(x, BF)


def _phi(t):
    return jnp.where(t > 0, t + 1.0, jnp.exp(t)) + 1e-6


def _half(i, n):
    return slice(i * n, (i + 1) * n)


def _form(name, blk):
    if name not in _SUMS:
        return blk(0 if name == "11" else 3)
    i, j, sign = _SUMS[name]
    a, b = blk(i).astype(F32), blk(j).astype(F32)
    return (a + b if sign > 0 else a - b).astype(BF)


def _operand(blk, keep=None, rows=slice(None)):
    kept = []

    def get(name):
        if name in kept:
            return keep[_SLOT[name], rows, :]
        v = _form(name, blk)
        if keep is not None and name in _SUMS:
            keep[_SLOT[name], rows, :] = v
            kept.append(name)
        return v
    return get


def _strassen(a, b, mul, emit, before=None):
    t = {}
    before = before or {}

    def m2(v):
        t["m2"] = v

    def m4(v):
        emit(1, 0, t["m2"] + v)
        t["c11"] = v

    def m5(v):
        t["c11"] = t["c11"] - v
        t["m5"] = v

    def m1(v):
        t["c11"] = t["c11"] + v
        t["c22"] = v - t["m2"]

    def m7(v):
        emit(0, 0, t["c11"] + v)

    def m3(v):
        emit(0, 1, v + t["m5"])
        t["c22"] = t["c22"] + v

    def m6(v):
        emit(1, 1, t["c22"] + v)

    def step(n, na, nb, use):
        def run():
            if n in before:
                before[n]()
            use(mul(a(na), b(nb)))
        return run

    return [step(2, "Q", "11", m2), step(4, "22", "T", m4), step(5, "R", "22", m5),
            step(1, "P", "P", m1), step(7, "U", "Q", m7), step(3, "11", "U", m3),
            step(6, "T", "R", m6)]


def _run(steps, tasks=()):
    done = 0
    for i, step in enumerate(steps):
        step()
        upto = (len(tasks) * (i + 1)) // len(steps)
        for task in tasks[done:upto]:
            task()
        done = upto


def _attention(k_s, q_s, vt_s, ot_s):
    nck = S // CK

    def heads(it, chk):
        h0 = it * HU
        g = h0 // 4
        items = [(u, c) for u in range(HU) for c in range(nck)]
        wq, m, l, acc = {}, {}, {}, {}

        def scores(u, c):
            if u not in wq:
                own = q_s[g, pl.ds(pl.multiple_of(((h0 + u) % 4) * 16, 16), 16), :]
                parts = [jnp.where(h0 % 4 + u == j, own, 0) if j % HU == u
                         else jnp.zeros((16, S), I32) for j in range(4)]
                wq[u] = _unpack(jnp.concatenate(parts, axis=0))
            return _dot(_unpack(k_s[g, _half(c, CK // 2), :]), wq[u])

        def probs(u, c, s):
            s = s.reshape(CK // 8, 8, S)
            if c == 0:
                m[u] = jnp.broadcast_to(jnp.max(s[0], axis=0, keepdims=True), (8, S))
            p = jnp.exp2(s - m[u][None])
            ls = jnp.sum(p, axis=0)
            l[u] = ls if c == 0 else l[u] + ls
            return p.reshape(CK, S).astype(BF)

        def values(u, c, pb, chk):
            rows = pl.ds(pl.multiple_of((h0 + u) * 16, 16), 16)
            a = _dot(_unpack(vt_s[rows, _half(c, CK)]), pb)
            acc[u] = a if c == 0 else acc[u] + a
            if c == nck - 1:
                lt = jnp.sum(l[u], axis=0, keepdims=True)
                o = acc[u] * (1.0 / lt)
                ot_s[rows, :] = _pack(o)
                chk = chk + jnp.sum(jnp.abs(o).reshape(DH // 8, 8, S), axis=0) + lt
            return chk

        s, pb = scores(*items[0]), None
        for i, item in enumerate(items):
            s_next = scores(*items[i + 1]) if i + 1 < len(items) else None
            if pb is not None:
                chk = values(*items[i - 1], pb, chk)
            pb = probs(*item, s)
            s = s_next
        return values(*items[-1], pb, chk)

    chk = jax.lax.fori_loop(0, H // HU, heads, jnp.zeros((8, S), F32))
    n_unsafe = jnp.sum(jnp.where(chk < _SAFE, 0.0, 1.0))

    @pl.when(n_unsafe > 0.0)
    def _with_true_max():
        sb = 512

        def body(it, _):
            h = it // (S // sb)
            rows = pl.ds(pl.multiple_of(h * 16, 16), 16)
            cols = pl.ds(pl.multiple_of((it % (S // sb)) * sb, sb), sb)
            own = (jax.lax.broadcasted_iota(I32, (64, sb), 0) >> 4) == h % 4
            wq = _unpack(jnp.where(own, q_s[h // 4, :, cols], 0))

            def scores(c):
                keys = pl.ds(pl.multiple_of(c * (CK // 2), CK // 2), CK // 2)
                return _dot(_unpack(k_s[h // 4, keys, :]), wq)

            def row_max(c, m):
                return jnp.maximum(m, jnp.max(scores(c), axis=0, keepdims=True))

            m = jax.lax.fori_loop(0, nck, row_max, jnp.full((1, sb), -jnp.inf, F32))

            def accumulate(c, carry):
                acc, l = carry
                p = jnp.exp2(scores(c) - m)
                vt = _unpack(vt_s[rows, pl.ds(pl.multiple_of(c * CK, CK), CK)])
                return acc + _dot(vt, p.astype(BF)), l + jnp.sum(p, axis=0, keepdims=True)

            acc, l = jax.lax.fori_loop(
                0, nck, accumulate, (jnp.zeros((DH, sb), F32), jnp.zeros((1, sb), F32)))
            ot_s[rows, cols] = _pack(acc / l)
            return 0

        jax.lax.fori_loop(0, (S // sb) * H, body, 0)


def _kernel(ax_h, aw_h, awo_h, bx_h, bw_h, bwo_h, out_h,
            xa, wa, woa, xb, wb, wob, k_s, q_s, wt0, wt1, ws0, ws1, ws2, xsa, xsb, os_s,
            vt_s, ot_s, m_s, z_s, y_s, in_sem, out_sem):
    lo, hi = _half(0, D2), _half(1, D2)

    def x_part(i, r):
        rows = pl.ds(i * S2 + r * RB, RB)
        return ax_h.at[0, rows, :], xa.at[rows, :]

    def w_part(rows, cols):
        return aw_h.at[rows, cols], wa.at[rows, cols]

    def wk_part(i, j):
        return w_part(pl.ds(i * D2, D2), pl.ds(D + j * D2, D2))

    parts = [("x10", x_part(1, 0)), ("k00", wk_part(0, 0)), ("k10", wk_part(1, 0))]
    parts += [(f"x1{r}", x_part(1, r)) for r in range(1, NRB)]
    parts += [("x00", x_part(0, 0)), ("k11", wk_part(1, 1)), ("k01", wk_part(0, 1))]
    parts += [(f"x0{r}", x_part(0, r)) for r in range(1, NRB)]
    parts += [("wq", w_part(slice(None), pl.ds(0, D))), ("wv", w_part(slice(None), pl.ds(2 * D, D))),
              ("wb", (bw_h, wb)), ("xb", (bx_h.at[0], xb)), ("woa", (awo_h, woa)), ("wob", (bwo_h, wob))]
    loads = {name: pltpu.make_async_copy(src, dst, in_sem.at[i])
             for i, (name, (src, dst)) in enumerate(parts)}
    for name, _ in parts:
        loads[name].start()

    def wait(*names):
        def run():
            for name in names:
                loads[name].wait()
        return run

    stores, retired = [], []

    def store_out(rows, cols, y):
        y_s[rows, cols] = y.astype(BF)
        cp = pltpu.make_async_copy(y_s.at[rows, cols], out_h.at[0, rows, cols],
                                   out_sem.at[len(stores)])
        cp.start()
        stores.append(cp)

    def retire():
        retired.append(stores[len(retired)])
        retired[-1].wait()

    def x_operands(x, keep):
        def one(r):
            def blk(i):
                r0 = (i // 2) * S2 + r * RB
                return x[r0:r0 + RB, _half(i % 2, D2)]
            return _operand(blk, keep, _half(r, RB))
        return [one(r) for r in range(NRB)]

    def w_operand(w, c0, keep):
        def blk(i):
            ca = c0 + (i % 2) * D2
            return w[_half(i // 2, D2), ca:ca + D2]
        return _operand(blk, keep)

    def wt_operand(wt, keep):
        return _operand(lambda i: wt[_half(i % 2, D2), _half(i // 2, D2)], keep)

    def transpose_tasks(wt, w, c0):
        def task(c, rows):
            def run():
                wt[c:c + TR, rows] = w[rows, c0 + c:c0 + c + TR].T
            return run
        return [task(c, _half(i, D2)) for c in range(0, D, TR) for i in range(2)]

    def operand_t_tasks(dst, blk, r0, r1):
        def task(r, name):
            def run():
                dst[_SLOT[name], r:r + TR, :] = _form(name, lambda i: blk(i, r)).T
            return run
        return [task(r, name) for r in range(r0, r1, TR) for name in _SLOT]

    def wt_tasks(dst, w, c0):
        def blk(i, r):
            ca = c0 + (i % 2) * D2 + r
            return w[_half(i // 2, D2), ca:ca + TR]
        return operand_t_tasks(dst, blk, 0, D2)

    def rows_tasks(src, r):
        def blk(i, c):
            ca = (i // 2) * S2 + c
            return _unpack(src[_half(i % 2, D2 // 2), ca:ca + TR])
        return operand_t_tasks(os_s, blk, r * RB, (r + 1) * RB) if r < NRB else []

    def tokens(i, r):
        return slice(i * S2 + r * RB, i * S2 + (r + 1) * RB)

    def project(x_ops, w_op, mul, emit, r, before=None):
        return _strassen(x_ops[r], w_op, mul, lambda i, j, v: emit(tokens(i, r), j, v), before)

    def out_steps(w_op, col0, r):
        def emit(i, j, v):
            store_out(pl.ds(i * S2 + r * RB, RB), pl.ds(col0 + j * D2, D2), v)
        return _strassen(lambda name: os_s[_SLOT[name], _half(r, RB), :], w_op, _dot, emit)

    def emit_k(tok, j, v):
        kp = _pack(v)
        for g in range(HG // 2):
            k_s[j * (HG // 2) + g, tok.start // 2:tok.stop // 2, :] = kp[:, _half(g, 128)]

    xa_ops = x_operands(xa, xsa)
    wk = w_operand(wa, D, ws0)
    k0 = project(xa_ops, wk, _dot, emit_k, 0, {2: wait("x10", "k00"), 4: wait("k10"),
                                               5: wait("x00", "k11", "k01", "x01")})
    k1 = project(xa_ops, wk, _dot, emit_k, 1, {2: wait("x11"), 4: wait("x12"),
                                               3: wait("x02", "x03", "wq")})
    k2 = project(xa_ops, wk, _dot, emit_k, 2, {4: wait("x13")})
    k3 = project(xa_ops, wk, _dot, emit_k, 3, {3: wait("wv")})
    _run(k0[:2] + k1[:2] + k2[:2] + k3[:2] + k0[2:] + k1[2:])
    _run(k2[2:] + k3[2:5], transpose_tasks(wt0, wa, 0))
    _run(k3[5:])

    def emit_q(tok, j, v):
        qp = _pack(v * _QSCALE)
        for g in range(HG // 2):
            q_s[j * (HG // 2) + g, :, tok] = qp[_half(g, 64), :]

    wq_t = wt_operand(wt0, ws1)
    _run([s for r in range(NRB) for s in project(xa_ops, wq_t, _dot_t, emit_q, r)],
         transpose_tasks(wt1, wa, 2 * D))

    def emit_v(tok, j, v):
        vt_s[_half(j, D2 // 2), tok] = _pack(v)

    wv_t = wt_operand(wt1, ws2)
    steps = [s for r in range(NRB) for s in project(xa_ops, wv_t, _dot_t, emit_v, r)]
    _run(steps[:8])
    wait("wb", "xb", "woa", "wob")()
    _run(steps[8:], wt_tasks(ws0, wb, D))

    _attention(k_s, q_s, vt_s, ot_s)

    pkt = vt_s
    zacc = [None, None]

    def emit_pk(tok, j, v):
        pk = _phi(v)
        pkt[_half(j, D2 // 2), tok] = _pack(pk)
        for t in range(RB // 128):
            u = pk[:, _half(t, 128)]
            zacc[j] = u if zacc[j] is None else zacc[j] + u

    def z_task(j):
        def run():
            z_s[_half(j, D2), :] = jnp.broadcast_to(
                jnp.sum(zacc[j], axis=1, keepdims=True), (D2, 128))
        return run

    xb_ops = x_operands(xb, xsb)
    _run([s for r in range(NRB)
          for s in project(xb_ops, lambda name: ws0[_SLOT[name]], _dot_t, emit_pk, r)],
         rows_tasks(ot_s, 0))

    wo_a = w_operand(woa, 0, ws1)
    for r in range(NRB):
        _run(out_steps(wo_a, 0, r),
             rows_tasks(ot_s, r + 1) + ([z_task(0), z_task(1)] if r == NRB - 1 else []))

    retire()
    g_s = wt0

    def xb_all(name):
        if name in _SUMS:
            return xsb[_SLOT[name]]
        return xb[0:S2, lo] if name == "11" else xb[S2:S, hi]

    def g_steps(r):
        def blk(i):
            pa = ((i // 2) * D2 + r * RB) // 2
            return _unpack(pkt[pa:pa + RB // 2, _half(i % 2, S2)])

        def emit(i, j, v):
            g_s[i * D2 + r * RB:i * D2 + (r + 1) * RB, _half(j, D2)] = v.astype(BF)
        return _strassen(_operand(blk), xb_all, _dot, emit)

    _run([s for r in range(D2 // RB) for s in g_steps(r)], wt_tasks(ws2, wb, 0))

    retire()
    kv_s = woa
    same_head = ((jax.lax.broadcasted_iota(I32, (128, 128), 0) >> 5)
                 == (jax.lax.broadcasted_iota(I32, (128, 128), 1) >> 5))
    for g in range(HG):
        kv = _dot(g_s[_half(g, 128), :], wb[:, _half(2 * HG + g, 128)])
        kv_s[_half(g, 128), 0:128] = jnp.where(same_head, kv, 0.0).astype(BF)
    for g in range(HG):
        rows = _half(g, 128)
        m_s[rows, :] = _dot(kv_s[rows, 0:128], wob[rows, :]).astype(BF)

    pqt = ot_s

    def emit_pq(tok, j, v):
        pq = _phi(v)
        z = z_s[_half(j, D2), :]
        for t in range(RB // 128):
            u = pq[:, _half(t, 128)]
            den = jnp.sum((u * z).reshape(H // 2, DH, 128), axis=1, keepdims=True) + 1e-6
            un = u.reshape(H // 2, DH, 128) * (1.0 / den)
            c0 = tok.start + t * 128
            pqt[_half(j, D2 // 2), c0:c0 + 128] = _pack(un.reshape(D2, 128))

    for r in range(NRB):
        _run(project(xb_ops, lambda name: ws2[_SLOT[name]], _dot_t, emit_pq, r),
             rows_tasks(pqt, 0) if r == 1 else [])

    retire()
    m_b = w_operand(m_s, 0, ws0)
    for r in range(NRB):
        _run(out_steps(m_b, D, r), rows_tasks(pqt, r + 1))

    while len(retired) < len(stores):
        retire()


@jax.jit
def pallas_concat_heads__mha_block__linear_attn_block__prompt_kernel(
    A_x: jax.Array,
    A_wqkv: jax.Array,
    A_wo: jax.Array,
    B_x: jax.Array,
    B_wqkv: jax.Array,
    B_wo: jax.Array,
):
    hbm = pl.BlockSpec(memory_space=pl.ANY)
    vmem = pltpu.VMEM
    return pl.pallas_call(
        _kernel,
        in_specs=[hbm] * 6,
        out_specs=hbm,
        out_shape=jax.ShapeDtypeStruct((1, S, 2 * D), BF),
        scratch_shapes=[
            vmem((S, D), BF), vmem((D, 3 * D), BF), vmem((D, D), BF),
            vmem((S, D), BF), vmem((D, 3 * D), BF), vmem((D, D), BF),
            vmem((HG, S2, 128), I32), vmem((HG, 64, S), I32),
            vmem((D, D), BF), vmem((D, D), BF),
            vmem((7, D2, D2), BF), vmem((5, D2, D2), BF), vmem((7, D2, D2), BF),
            vmem((5, S2, D2), BF), vmem((5, S2, D2), BF), vmem((7, S2, D2), BF),
            vmem((D2, S), I32), vmem((D2, S), I32),
            vmem((D, D), BF), vmem((D, 128), F32),
            vmem((S, 2 * D), BF),
            pltpu.SemaphoreType.DMA((2 * NRB + 10,)),
            pltpu.SemaphoreType.DMA((8 * NRB,)),
        ],
        compiler_params=pltpu.CompilerParams(vmem_limit_bytes=110 * 2 ** 20),
    )(A_x, A_wqkv, A_wo, B_x, B_wqkv, B_wo)
```
